```python
import jax
import jax.numpy as jnp

def _softmax(x, axis=-1):
    return jax.nn.softmax(x, axis=axis)

def _gelu(x):
    return jax.nn.gelu(x, approximate=True)

def _silu(x):
    return jax.nn.silu(x)

def _sigmoid(x):
    return jax.nn.sigmoid(x)

def _layernorm(x, axis=-1, eps=1e-05):
    m = jnp.mean(x, axis=axis, keepdims=True)
    v = jnp.var(x, axis=axis, keepdims=True)
    return (x - m) / jnp.sqrt(v + eps)

def _scatter_add(tgt, idx, src, axis=0):
    return tgt.at[idx].add(src)

def _segment_sum(src, seg, n):
    return jax.ops.segment_sum(src, seg, n)

class _Rng:

    def __init__(self, key):
        self._k = key

    def _next(self):
        self._k, sub = jax.random.split(self._k)
        return sub

    def normal(self, shape):
        return jax.random.normal(self._next(), shape, dtype=jnp.bfloat16)

    def randint(self, lo, hi, shape):
        return jax.random.randint(self._next(), shape, lo, hi, dtype=jnp.int32)

    def uniform(self, shape, lo=0.0, hi=1.0):
        return jax.random.uniform(self._next(), shape, jnp.bfloat16, lo, hi)

    def permutation(self, n):
        return jax.random.permutation(self._next(), n)
kernel_name = 'adaLN_cond__sliding_block_cached__glu_gated_glu__decode'

def setup_inputs():
    _rng = _Rng(jax.random.key(int.from_bytes(__import__("os").urandom(4), "little")))
    _w = lambda a: (lambda t: t.astype(jnp.bfloat16) if jnp.issubdtype(t.dtype, jnp.floating) else t)(jnp.asarray(a))

    def _A_setup():
        B, Sq, D = (8, 1, 512)
        Hq, Hkv, Sk, Dh = (32, 32, 4096, 128)
        assert Hq % Hkv == 0, (Hq, Hkv)
        return {'x': _w((lambda *s: _rng.normal(s) * 0.05)(B, Sq, D)), 'k_cache': _w((lambda *s: _rng.normal(s) * 0.05)(B, Hkv, Sk, Dh)), 'v_cache': _w((lambda *s: _rng.normal(s) * 0.05)(B, Hkv, Sk, Dh)), 'wq': _w((lambda *s: _rng.normal(s) * 0.05)(D, Hq * Dh) * D ** (-0.5)), 'wo': _w((lambda *s: _rng.normal(s) * 0.05)(Hq * Dh, D) * (Hq * Dh) ** (-0.5))}
    _A_in = _A_setup()

    def _B_setup():
        B, S, D, F = (8, 1, 512, 1376)
        return {'x': _w((lambda *s: _rng.normal(s) * 0.05)(B, S, D)), 'w_gate': _w((lambda *s: _rng.normal(s) * 0.05)(D, F)), 'w_up': _w((lambda *s: _rng.normal(s) * 0.05)(D, F)), 'w_down': _w((lambda *s: _rng.normal(s) * 0.05)(F, D))}
    _B_in = _B_setup()
    return {'A_x': _A_in['x'], 'A_k_cache': _A_in['k_cache'], 'A_v_cache': _A_in['v_cache'], 'A_wq': _A_in['wq'], 'A_wo': _A_in['wo'], 'B_x': _B_in['x'], 'B_w_gate': _B_in['w_gate'], 'B_w_up': _B_in['w_up'], 'B_w_down': _B_in['w_down'], 'c': _w((lambda *s: _rng.normal(s) * 0.05)(8, 512)), 'w_mod': _w((lambda *s: _rng.normal(s) * 0.05)(512, 6 * 512) * 512 ** (-0.5))}

def reference(A_x, A_k_cache, A_v_cache, A_wq, A_wo, B_x, B_w_gate, B_w_up, B_w_down, c, w_mod):

    def _A_ref(x, k_cache, v_cache, wq, wo):
        B, Sq, D = x.shape
        Hq, Dh = (32, 128)
        Hkv, Sk = (k_cache.shape[1], k_cache.shape[2])
        W = min(4096, max(256, Sk // 4))
        rep = Hq // Hkv
        q = (lambda x, *d: x.transpose(*d))((x @ wq).reshape(B, Sq, Hq, Dh), 0, 2, 1, 3)
        k = jnp.repeat(k_cache[:, :, Sk - W:, :], rep, axis=1)
        v = jnp.repeat(v_cache[:, :, Sk - W:, :], rep, axis=1)
        scores = jnp.einsum('bhqd,bhkd->bhqk', q, k) * Dh ** (-0.5)
        p = _softmax(scores, axis=-1)
        o = jnp.einsum('bhqk,bhkd->bhqd', p, v)
        return (lambda x, *d: x.transpose(*d))(o, 0, 2, 1, 3).reshape(B, Sq, Hq * Dh) @ wo

    def _B_ref(x, w_gate, w_up, w_down):
        g = jnp.einsum('bsd,df->bsf', x, w_gate)
        u = jnp.einsum('bsd,df->bsf', x, w_up)
        h = _sigmoid(g) * u
        return jnp.einsum('bsf,fd->bsd', h, w_down)
    x = A_x
    mod = (_silu(c) @ w_mod).reshape(c.shape[0], 6, 1, -1)
    sa, ca, ga, sb, cb, gb = (mod[:, 0].copy(), mod[:, 1].copy(), mod[:, 2].copy(), mod[:, 3].copy(), mod[:, 4].copy(), mod[:, 5].copy())
    h = _layernorm(x, axis=-1) * (1 + ca) + sa
    x = x + ga * _A_ref(h, A_k_cache, A_v_cache, A_wq, A_wo)
    h = _layernorm(x, axis=-1) * (1 + cb) + sb
    x = x + gb * _B_ref(h, B_w_gate, B_w_up, B_w_down)
    return x
```

```python
import functools
import jax, jax.numpy as jnp, numpy as np
from jax.experimental import pallas as pl
from jax.experimental.pallas import tpu as pltpu

B, D, HQ, DH, SK, W, F = 8, 512, 32, 128, 4096, 1024, 1376
bf = jnp.bfloat16
f32 = jnp.float32
NT = (((1,), (1,)), ((), ()))
NN = (((1,), (0,)), ((), ()))

def _ln(x):
    m = jnp.mean(x, axis=-1, keepdims=True)
    xc = x - m
    v = jnp.mean(xc * xc, axis=-1, keepdims=True)
    return xc / jnp.sqrt(v + 1e-5)

def _make(depth=3):
    def kernel(x_h, k_h, v_h, wq_h, wo_h, wg_h, wu_h, wd_h, c_h, wm_h, out_h,
               x_v, c_v, wm_v, wq_v, wo_v, wg_v, wu_v, wd_v, kbuf, vbuf, q_s, o_s, out_v,
               sem_w, sem_k, sem_v, sem_o):
        cp_x = pltpu.make_async_copy(x_h, x_v, sem_w.at[0])
        cp_c = pltpu.make_async_copy(c_h, c_v, sem_w.at[1])
        cp_wm = pltpu.make_async_copy(wm_h, wm_v, sem_w.at[2])
        cp_wq = pltpu.make_async_copy(wq_h, wq_v, sem_w.at[3])
        cp_wo = pltpu.make_async_copy(wo_h, wo_v, sem_w.at[4])
        cp_wg = pltpu.make_async_copy(wg_h, wg_v, sem_w.at[5])
        cp_wu = pltpu.make_async_copy(wu_h, wu_v, sem_w.at[6])
        cp_wd = pltpu.make_async_copy(wd_h, wd_v, sem_w.at[7])

        def kcp(h, slot):
            return pltpu.make_async_copy(k_h.at[:, h, pl.ds(SK - W, W), :], kbuf.at[slot], sem_k.at[slot])
        def vcp(h, slot):
            return pltpu.make_async_copy(v_h.at[:, h, pl.ds(SK - W, W), :], vbuf.at[slot], sem_v.at[slot])

        cp_x.start(); cp_c.start(); cp_wm.start(); cp_wq.start()
        for s in range(depth):
            kcp(s, s).start(); vcp(s, s).start()

        cp_c.wait(); cp_wm.wait()
        c = c_v[...].astype(f32)
        sc = (c * jax.nn.sigmoid(c)).astype(bf)
        mod = jnp.dot(sc, wm_v[...], preferred_element_type=f32)
        cp_x.wait()
        x = x_v[...].astype(f32)
        sa, ca = mod[:, 0:D], mod[:, D:2*D]
        h1 = (_ln(x) * (1.0 + ca) + sa).astype(bf)
        cp_wq.wait()
        q = jnp.dot(h1, wq_v[...], preferred_element_type=f32) * (DH ** -0.5)
        qb = q.astype(bf)
        for h in range(HQ):
            q_s[h] = qb[:, h*DH:(h+1)*DH]

        row = jax.lax.broadcasted_iota(jnp.int32, (B, 1), 0)

        def body(h, _):
            slot = h % depth
            kcp(h, slot).wait()
            qh = q_s[h]
            s = None
            for b in range(B):
                sb = jax.lax.dot_general(qh, kbuf[slot, b], NT, preferred_element_type=f32)
                s = sb if s is None else jnp.where(row == b, sb, s)
            @pl.when(h + depth < HQ)
            def _():
                kcp(h + depth, slot).start()
            m = jnp.max(s, axis=-1, keepdims=True)
            e = jnp.exp(s - m)
            l = jnp.sum(e, axis=-1, keepdims=True)
            p = e.astype(bf)
            vcp(h, slot).wait()
            o = None
            for b in range(B):
                ob = jnp.dot(p, vbuf[slot, b], preferred_element_type=f32)
                o = ob if o is None else jnp.where(row == b, ob, o)
            @pl.when(h + depth < HQ)
            def _():
                vcp(h + depth, slot).start()
            @pl.when(h + depth == HQ)
            def _():
                cp_wo.start(); cp_wg.start(); cp_wu.start(); cp_wd.start()
            o_s[h] = (o / l).astype(bf)
            return 0
        jax.lax.fori_loop(0, HQ, body, 0)

        cp_wo.wait()
        acc = None
        for h in range(HQ):
            t = jnp.dot(o_s[h], wo_v[pl.ds(h*DH, DH), :], preferred_element_type=f32)
            acc = t if acc is None else acc + t
        ga, sb_, cb, gb = mod[:, 2*D:3*D], mod[:, 3*D:4*D], mod[:, 4*D:5*D], mod[:, 5*D:6*D]
        x2 = x + ga * acc
        h2 = (_ln(x2) * (1.0 + cb) + sb_).astype(bf)
        cp_wg.wait()
        g = jax.lax.dot_general(h2, wg_v[...], NT, preferred_element_type=f32)
        cp_wu.wait()
        u = jax.lax.dot_general(h2, wu_v[...], NT, preferred_element_type=f32)
        hh = (jax.nn.sigmoid(g) * u).astype(bf)
        cp_wd.wait()
        dn = jnp.dot(hh, wd_v[...], preferred_element_type=f32)
        out_v[...] = (x2 + gb * dn).astype(bf)
        oc = pltpu.make_async_copy(out_v, out_h, sem_o)
        oc.start(); oc.wait()

    def f(A_x, A_k_cache, A_v_cache, A_wq, A_wo, B_x, B_w_gate, B_w_up, B_w_down, c, w_mod):
        out = pl.pallas_call(kernel,
            in_specs=[pl.BlockSpec(memory_space=pltpu.HBM)]*10,
            out_specs=pl.BlockSpec(memory_space=pltpu.HBM),
            out_shape=jax.ShapeDtypeStruct((B, D), bf),
            scratch_shapes=[
                pltpu.VMEM((B, D), bf), pltpu.VMEM((B, D), bf), pltpu.VMEM((D, 6*D), bf),
                pltpu.VMEM((D, HQ*DH), bf), pltpu.VMEM((HQ*DH, D), bf),
                pltpu.VMEM((F, D), bf), pltpu.VMEM((F, D), bf), pltpu.VMEM((F, D), bf),
                pltpu.VMEM((depth, B, W, DH), bf), pltpu.VMEM((depth, B, W, DH), bf),
                pltpu.VMEM((HQ, B, DH), bf), pltpu.VMEM((HQ, B, DH), bf), pltpu.VMEM((B, D), bf),
                pltpu.SemaphoreType.DMA((8,)), pltpu.SemaphoreType.DMA((depth,)), pltpu.SemaphoreType.DMA((depth,)),
                pltpu.SemaphoreType.DMA(())],
            compiler_params=pltpu.CompilerParams(vmem_limit_bytes=100*2**20),
        )(A_x.reshape(B, D), A_k_cache, A_v_cache, A_wq, A_wo, B_w_gate.T, B_w_up.T, B_w_down, c, w_mod)
        return out.reshape(B, 1, D)
    return f


@jax.jit
def pallas_adaLN_cond__sliding_block_cached__glu_gated_glu__decode_kernel(
    A_x, A_k_cache, A_v_cache, A_wq, A_wo, B_x, B_w_gate, B_w_up, B_w_down, c, w_mod,
):
    return _make(3)(A_x, A_k_cache, A_v_cache, A_wq, A_wo, B_x, B_w_gate, B_w_up, B_w_down, c, w_mod)
```

```python
import jax
import jax.numpy as jnp
import jax.experimental.pallas as pl
import jax.experimental.pallas.tpu as pltpu

B, D, HQ, DH, SK, F = 8, 512, 32, 128, 4096, 1376
W = min(4096, max(256, SK // 4))
HG = 8
NG = HQ // HG
NS = B * NG
NR = 128
WR = 32
N_WO = 4
WD_B = (0, 768, 1152, F)

S_X, S_C, S_WM, S_WQ, S_WG, S_WU, S_WO = range(7)
S_WD = S_WO + N_WO
N_WSEM = S_WD + len(WD_B) - 1

BF16, F32 = jnp.bfloat16, jnp.float32
NT = (((1,), (1,)), ((), ()))


def _layernorm(x):
    m = jnp.mean(x, axis=-1, keepdims=True)
    xc = x - m
    v = jnp.mean(xc * xc, axis=-1, keepdims=True)
    return xc / jnp.sqrt(v + 1e-5)


def _spread(items, n=4):
    per = -(-len(items) // n)
    return [items[i] for i in sorted(range(len(items)), key=lambda i: (i % per, i))]


class _Stream:
    def __init__(self, items):
        self.items, self.pos = list(items), 0

    def issue(self, count=None):
        left = len(self.items) - self.pos
        for _ in range(left if count is None else min(count, left)):
            src, dst, sem, prio = self.items[self.pos]
            pltpu.make_async_copy(src, dst, sem).start(priority=prio)
            self.pos += 1

    def issue_to(self, pos):
        self.issue(pos - self.pos)


def _alternate(items):
    return [it + (i % 2,) for i, it in enumerate(items)]


def _kernel(x_h, k_h, v_h, wq_h, wo_h, wg_h, wu_h, wd_h, c_h, wm_h, out_h,
            x_v, c_v, wm_v, wq_v, wo_v, wg_v, wu_v, wd_v, kbuf, vbuf, q_s, o_s, out_v,
            sem_w, sem_k, sem_v, sem_o):

    def pieces(src, dst, si, rows, cols, r_lo=0, r_hi=None):
        r_hi = src.shape[0] if r_hi is None else r_hi
        tiles = [(r, c) for r in range(r_lo, r_hi, rows) for c in range(0, src.shape[1], cols)]
        return [(src.at[pl.ds(r, rows), pl.ds(c, cols)], dst.at[pl.ds(r, rows), pl.ds(c, cols)],
                 sem_w.at[si]) for r, c in _spread(tiles)]

    def kv_pieces(j, slot):
        b, h0 = j // NG, (j % NG) * HG
        out = []
        for r in range(W // NR):
            rows = pl.ds(SK - W + r * NR, NR)
            for i in range(HG):
                out.append((k_h.at[b, h0 + i, rows, :], kbuf.at[slot, i, pl.ds(r * NR, NR), :],
                            sem_k.at[slot], 0))
                out.append((v_h.at[b, h0 + i, rows, :], vbuf.at[slot, i, pl.ds(r * NR, NR), :],
                            sem_v.at[slot], 1))
        return out

    def wait(dst, sem):
        pltpu.make_async_copy(dst, dst, sem).wait()

    def dot(a, b):
        return jnp.dot(a, b, preferred_element_type=F32)

    def dot_nt(a, b):
        return jax.lax.dot_general(a, b, NT, preferred_element_type=F32)

    row = jax.lax.broadcasted_iota(jnp.int32, (HG, 1), 0)

    def step_rows(j):
        return pl.ds(j * HG, HG) if isinstance(j, int) else pl.ds(pl.multiple_of(j * HG, HG), HG)

    def scores(j, slot):
        wait(kbuf.at[slot], sem_k.at[slot])
        q = q_s[step_rows(j), :].astype(BF16)
        s = None
        for i in range(HG):
            si = dot_nt(q, kbuf[slot, i])
            s = si if s is None else jnp.where(row == i, si, s)
        e = jnp.exp(s - jnp.max(s, axis=-1, keepdims=True))
        return e.astype(BF16), jnp.sum(e, axis=-1, keepdims=True)

    def values(j, slot, p, l):
        wait(vbuf.at[slot], sem_v.at[slot])
        o = None
        for i in range(HG):
            oi = dot(p, vbuf[slot, i])
            o = oi if o is None else jnp.where(row == i, oi, o)
        o_s[step_rows(j), :] = o / l

    LAG = 128
    wm = _alternate(pieces(wm_h, wm_v, S_WM, 16, 1024))
    wq = _alternate(pieces(wq_h, wq_v, S_WQ, 8, 2048))
    st = _Stream([(c_h, c_v, sem_w.at[S_C], 0), (x_h, x_v, sem_w.at[S_X], 1)]
                 + wm + wq + kv_pieces(0, 0) + kv_pieces(1, 1))
    st.issue_to(2 + len(wm) + LAG)
    wait(c_v, sem_w.at[S_C])
    wait(x_v, sem_w.at[S_X])
    wait(wm_v, sem_w.at[S_WM])
    c = c_v[...].astype(F32)
    mod = dot((c * jax.nn.sigmoid(c)).astype(BF16), wm_v[...])
    sa, ca, ga, sb, cb, gb = (mod[:, i * D:(i + 1) * D] for i in range(6))
    x = x_v[...].astype(F32)
    h = (_layernorm(x) * (1.0 + ca) + sa).astype(BF16)
    st.issue_to(2 + len(wm) + len(wq) + LAG)
    wait(wq_v, sem_w.at[S_WQ])
    q = dot(h, wq_v[...]) * (DH ** -0.5)
    for hd in range(HQ):
        q_s[pl.ds(hd, B, stride=HQ), :] = q[:, hd * DH:(hd + 1) * DH]
    st.issue()

    def body(j, carry):
        slot = j % 2
        values(j, slot, *scores(j, slot))
        _Stream(kv_pieces(j + 2, slot)).issue()
        return carry

    jax.lax.fori_loop(0, NS - 2, body, 0)

    rw = HQ * DH // N_WO
    wo = [pieces(wo_h, wo_v, S_WO + g, WR, D, g * rw, (g + 1) * rw) for g in range(N_WO)]
    wg = pieces(wg_h, wg_v, S_WG, WR, D)
    wu = pieces(wu_h, wu_v, S_WU, WR, D)
    wd = [pieces(wd_h, wd_v, S_WD + p, WR, D, WD_B[p], WD_B[p + 1]) for p in range(len(WD_B) - 1)]
    fast = [it + (0,) for g in wo + [wg] for it in g[0::2]] + [it + (0,) for it in wu]
    slow = [it + (1,) for g in wo + [wg] for it in g[1::2]] + [it + (1,) for g in wd for it in g]
    assert len(fast) == len(slow) + 1
    st = _Stream([it for pair in zip(fast, slow) for it in pair] + fast[-1:])

    values(NS - 2, NS % 2, *scores(NS - 2, NS % 2))
    st.issue(64)
    p, l = scores(NS - 1, (NS - 1) % 2)
    st.issue(64)
    values(NS - 1, (NS - 1) % 2, p, l)
    st.issue(32)

    attn = None
    for g, more in zip(range(N_WO), (32, 32, 20, None)):
        wait(wo_v.at[pl.ds(g * rw, rw)], sem_w.at[S_WO + g])
        for hd in range(g * rw // DH, (g + 1) * rw // DH):
            o = o_s[pl.ds(hd, B, stride=HQ), :].astype(BF16)
            t = dot(o, wo_v[pl.ds(hd * DH, DH), :])
            attn = t if attn is None else attn + t
        st.issue(more)
    x = x + ga * attn
    h = (_layernorm(x) * (1.0 + cb) + sb).astype(BF16)

    wait(wg_v, sem_w.at[S_WG])
    g = dot_nt(h, wg_v[...])
    wait(wu_v, sem_w.at[S_WU])
    hh = (jax.nn.sigmoid(g) * dot_nt(h, wu_v[...])).astype(BF16)
    down = None
    for p in range(len(WD_B) - 1):
        rows = pl.ds(WD_B[p], WD_B[p + 1] - WD_B[p])
        wait(wd_v.at[rows], sem_w.at[S_WD + p])
        t = dot(hh[:, WD_B[p]:WD_B[p + 1]], wd_v[rows, :])
        down = t if down is None else down + t
    out_v[...] = (x + gb * down).astype(BF16)
    out = pltpu.make_async_copy(out_v, out_h, sem_o)
    out.start()
    out.wait()


@jax.jit
def pallas_adaLN_cond__sliding_block_cached__glu_gated_glu__decode_kernel(
    A_x: jax.Array,
    A_k_cache: jax.Array,
    A_v_cache: jax.Array,
    A_wq: jax.Array,
    A_wo: jax.Array,
    B_x: jax.Array,
    B_w_gate: jax.Array,
    B_w_up: jax.Array,
    B_w_down: jax.Array,
    c: jax.Array,
    w_mod: jax.Array,
):
    del B_x
    assert A_x.shape == (B, 1, D) and A_k_cache.shape == A_v_cache.shape == (B, HQ, SK, DH)
    assert B_w_gate.shape == B_w_up.shape == (D, F) and B_w_down.shape == (F, D)
    hbm = pl.BlockSpec(memory_space=pltpu.HBM)
    vmem = lambda *shape, dtype=BF16: pltpu.VMEM(shape, dtype)
    dma = pltpu.SemaphoreType.DMA
    out = pl.pallas_call(
        _kernel,
        in_specs=[hbm] * 10,
        out_specs=hbm,
        out_shape=jax.ShapeDtypeStruct((B, D), BF16),
        scratch_shapes=[
            vmem(B, D), vmem(B, D), vmem(D, 6 * D), vmem(D, HQ * DH), vmem(HQ * DH, D),
            vmem(F, D), vmem(F, D), vmem(F, D),
            vmem(2, HG, W, DH), vmem(2, HG, W, DH),
            vmem(B * HQ, DH, dtype=F32), vmem(B * HQ, DH, dtype=F32), vmem(B, D),
            dma((N_WSEM,)), dma((2,)), dma((2,)), dma(()),
        ],
        compiler_params=pltpu.CompilerParams(
            vmem_limit_bytes=64 * 2**20, disable_bounds_checks=True),
    )(
        A_x.reshape(B, D), A_k_cache, A_v_cache, A_wq, A_wo,
        B_w_gate.T, B_w_up.T, B_w_down, c, w_mod,
    )
    return out.reshape(B, 1, D)
```

```python
import jax
import jax.numpy as jnp
import jax.experimental.pallas as pl
import jax.experimental.pallas.tpu as pltpu

B, D, HQ, DH, SK, F = 8, 512, 32, 128, 4096, 1376
W = min(4096, max(256, SK // 4))
HG = 8
SS = 16
NS = B * HQ // HG
NR = 128
K_SHIFT = NR // 2
WR = 32
N_WO = 4
WD_B = (0, 768, 1152, F)

S_X, S_C, S_WM, S_WQ, S_WG, S_WU, S_WO = range(7)
S_WD = S_WO + N_WO
N_WSEM = S_WD + len(WD_B) - 1

BF16, F32 = jnp.bfloat16, jnp.float32
NT = (((1,), (1,)), ((), ()))


def _layernorm(x):
    m = jnp.mean(x, axis=-1, keepdims=True)
    xc = x - m
    v = jnp.mean(xc * xc, axis=-1, keepdims=True)
    return xc / jnp.sqrt(v + 1e-5)


def _spread(items, n=4):
    per = -(-len(items) // n)
    return [items[i] for i in sorted(range(len(items)), key=lambda i: (i % per, i))]


def _cuts(total, size, shift):
    edges = [0] + list(range(shift or size, total, size)) + [total]
    return [(lo, hi - lo) for lo, hi in zip(edges, edges[1:])]


def _merge(a, b):
    keyed = [(i * len(b), 0, it) for i, it in enumerate(a)]
    keyed += [(i * len(a), 1, it) for i, it in enumerate(b)]
    return [it for _, _, it in sorted(keyed, key=lambda t: t[:2])]


class _Stream:
    def __init__(self, items):
        self.items, self.pos = list(items), 0

    def issue(self, count=None):
        left = len(self.items) - self.pos
        for _ in range(left if count is None else min(count, left)):
            src, dst, sem, prio = self.items[self.pos]
            pltpu.make_async_copy(src, dst, sem).start(priority=prio)
            self.pos += 1

    def issue_to(self, pos):
        self.issue(pos - self.pos)


def _alternate(items):
    return [it + (i % 2,) for i, it in enumerate(items)]


def _kernel(x_h, k_h, v_h, wq_h, wo_h, wg_h, wu_h, wd_h, c_h, wm_h, out_h,
            x_v, c_v, wm_v, wq_v, wo_v, wg_v, wu_v, wd_v, kbuf, vbuf, q_s, o_s, out_v,
            sem_w, sem_k, sem_v, sem_o):

    def pieces(src, dst, si, rows, cols, r_lo=0, r_hi=None):
        r_hi = src.shape[0] if r_hi is None else r_hi
        tiles = [(r, c) for r in range(r_lo, r_hi, rows) for c in range(0, src.shape[1], cols)]
        return [(src.at[pl.ds(r, rows), pl.ds(c, cols)], dst.at[pl.ds(r, rows), pl.ds(c, cols)],
                 sem_w.at[si]) for r, c in _spread(tiles)]

    def first_pair(j):
        return (j // SS) * (HG * SS) + j % SS

    def kv_pieces(j, slot):
        def copies(src, buf, sem, shift, prio):
            out = []
            for r, n in _cuts(W, NR, shift):
                for i in range(HG):
                    bh = first_pair(j) + i * SS
                    out.append((src.at[bh // HQ, bh % HQ, pl.ds(SK - W + r, n), :],
                                buf.at[slot, i, pl.ds(r, n), :], sem.at[slot], prio))
            return out
        return _merge(copies(k_h, kbuf, sem_k, K_SHIFT, 0), copies(v_h, vbuf, sem_v, 0, 1))

    def wait(dst, sem):
        pltpu.make_async_copy(dst, dst, sem).wait()

    def dot(a, b):
        return jnp.dot(a, b, preferred_element_type=F32)

    def dot_nt(a, b):
        return jax.lax.dot_general(a, b, NT, preferred_element_type=F32)

    row = jax.lax.broadcasted_iota(jnp.int32, (HG, 1), 0)

    def step_rows(j):
        return pl.ds(first_pair(j), HG, stride=SS)

    def scores(j, slot):
        wait(kbuf.at[slot], sem_k.at[slot])
        q = q_s[step_rows(j), :].astype(BF16)
        s = None
        for i in range(HG):
            si = dot_nt(q, kbuf[slot, i])
            s = si if s is None else jnp.where(row == i, si, s)
        e = jnp.exp(s - jnp.max(s, axis=-1, keepdims=True))
        return e.astype(BF16), jnp.sum(e, axis=-1, keepdims=True)

    def values(j, slot, p, l):
        wait(vbuf.at[slot], sem_v.at[slot])
        o = None
        for i in range(HG):
            oi = dot(p, vbuf[slot, i])
            o = oi if o is None else jnp.where(row == i, oi, o)
        o_s[step_rows(j), :] = o / l

    LAG = 128
    wm = _alternate(pieces(wm_h, wm_v, S_WM, 8, 1024))
    wq = _alternate(pieces(wq_h, wq_v, S_WQ, 8, 2048))
    st = _Stream([(c_h, c_v, sem_w.at[S_C], 0), (x_h, x_v, sem_w.at[S_X], 1)]
                 + wm + wq + kv_pieces(0, 0) + kv_pieces(1, 1))
    st.issue_to(2 + len(wm) + LAG)
    wait(c_v, sem_w.at[S_C])
    wait(x_v, sem_w.at[S_X])
    wait(wm_v, sem_w.at[S_WM])
    c = c_v[...].astype(F32)
    mod = dot((c * jax.nn.sigmoid(c)).astype(BF16), wm_v[...])
    sa, ca, ga, sb, cb, gb = (mod[:, i * D:(i + 1) * D] for i in range(6))
    x = x_v[...].astype(F32)
    h = (_layernorm(x) * (1.0 + ca) + sa).astype(BF16)
    st.issue_to(2 + len(wm) + len(wq) + LAG)
    wait(wq_v, sem_w.at[S_WQ])
    q = dot(h, wq_v[...]) * (DH ** -0.5)
    for hd in range(HQ):
        q_s[pl.ds(hd, B, stride=HQ), :] = q[:, hd * DH:(hd + 1) * DH]
    st.issue()

    def body(j, carry):
        slot = j % 2
        values(j, slot, *scores(j, slot))
        _Stream(kv_pieces(j + 2, slot)).issue()
        return carry

    jax.lax.fori_loop(0, NS - 2, body, 0)

    rw = HQ * DH // N_WO
    wo = [pieces(wo_h, wo_v, S_WO + g, WR, D, g * rw, (g + 1) * rw) for g in range(N_WO)]
    wg = pieces(wg_h, wg_v, S_WG, WR, D)
    wu = pieces(wu_h, wu_v, S_WU, WR, D)
    wd = [pieces(wd_h, wd_v, S_WD + p, WR, D, WD_B[p], WD_B[p + 1]) for p in range(len(WD_B) - 1)]
    fast = [it + (0,) for g in wo + [wg] for it in g[0::2]] + [it + (0,) for it in wu]
    slow = [it + (1,) for g in wo + [wg] for it in g[1::2]] + [it + (1,) for g in wd for it in g]
    assert len(fast) == len(slow) + 1
    st = _Stream([it for pair in zip(fast, slow) for it in pair] + fast[-1:])

    values(NS - 2, NS % 2, *scores(NS - 2, NS % 2))
    st.issue(64)
    p, l = scores(NS - 1, (NS - 1) % 2)
    st.issue(64)
    values(NS - 1, (NS - 1) % 2, p, l)
    st.issue(32)

    attn = None
    for g, more in zip(range(N_WO), (32, 32, 20, None)):
        wait(wo_v.at[pl.ds(g * rw, rw)], sem_w.at[S_WO + g])
        for hd in range(g * rw // DH, (g + 1) * rw // DH):
            o = o_s[pl.ds(hd, B, stride=HQ), :].astype(BF16)
            t = dot(o, wo_v[pl.ds(hd * DH, DH), :])
            attn = t if attn is None else attn + t
        st.issue(more)
    x = x + ga * attn
    h = (_layernorm(x) * (1.0 + cb) + sb).astype(BF16)

    wait(wg_v, sem_w.at[S_WG])
    g = dot_nt(h, wg_v[...])
    wait(wu_v, sem_w.at[S_WU])
    hh = (jax.nn.sigmoid(g) * dot_nt(h, wu_v[...])).astype(BF16)
    down = None
    for p in range(len(WD_B) - 1):
        rows = pl.ds(WD_B[p], WD_B[p + 1] - WD_B[p])
        wait(wd_v.at[rows], sem_w.at[S_WD + p])
        t = dot(hh[:, WD_B[p]:WD_B[p + 1]], wd_v[rows, :])
        down = t if down is None else down + t
    out_v[...] = (x + gb * down).astype(BF16)
    out = pltpu.make_async_copy(out_v, out_h, sem_o)
    out.start()
    out.wait()


@jax.jit
def pallas_adaLN_cond__sliding_block_cached__glu_gated_glu__decode_kernel(
    A_x: jax.Array,
    A_k_cache: jax.Array,
    A_v_cache: jax.Array,
    A_wq: jax.Array,
    A_wo: jax.Array,
    B_x: jax.Array,
    B_w_gate: jax.Array,
    B_w_up: jax.Array,
    B_w_down: jax.Array,
    c: jax.Array,
    w_mod: jax.Array,
):
    del B_x
    assert A_x.shape == (B, 1, D) and A_k_cache.shape == A_v_cache.shape == (B, HQ, SK, DH)
    assert B_w_gate.shape == B_w_up.shape == (D, F) and B_w_down.shape == (F, D)
    hbm = pl.BlockSpec(memory_space=pltpu.HBM)
    vmem = lambda *shape, dtype=BF16: pltpu.VMEM(shape, dtype)
    dma = pltpu.SemaphoreType.DMA
    out = pl.pallas_call(
        _kernel,
        in_specs=[hbm] * 10,
        out_specs=hbm,
        out_shape=jax.ShapeDtypeStruct((B, D), BF16),
        scratch_shapes=[
            vmem(B, D), vmem(B, D), vmem(D, 6 * D), vmem(D, HQ * DH), vmem(HQ * DH, D),
            vmem(F, D), vmem(F, D), vmem(F, D),
            vmem(2, HG, W, DH), vmem(2, HG, W, DH),
            vmem(B * HQ, DH, dtype=F32), vmem(B * HQ, DH, dtype=F32), vmem(B, D),
            dma((N_WSEM,)), dma((2,)), dma((2,)), dma(()),
        ],
        compiler_params=pltpu.CompilerParams(
            vmem_limit_bytes=64 * 2**20, disable_bounds_checks=True),
    )(
        A_x.reshape(B, D), A_k_cache, A_v_cache, A_wq, A_wo,
        B_w_gate.T, B_w_up.T, B_w_down, c, w_mod,
    )
    return out.reshape(B, 1, D)
```

```python
import jax
import jax.numpy as jnp
import jax.experimental.pallas as pl
import jax.experimental.pallas.tpu as pltpu

B, D, HQ, DH, SK, F = 8, 512, 32, 128, 4096, 1376
W = min(4096, max(256, SK // 4))
HG = 8
SS = 16
NS = B * HQ // HG
NR = 128
K_SHIFT = NR // 2
WR = 32
N_WO = 4
WU_B = (0, 768, F)
WD_B = (0, 640, 896, 1152, F)

S_X, S_C, S_WM, S_WQ, S_WG, S_WO = range(6)
S_WU = S_WO + N_WO
S_WD = S_WU + len(WU_B) - 1
N_WSEM = S_WD + len(WD_B) - 1

BF16, F32 = jnp.bfloat16, jnp.float32
NT = (((1,), (1,)), ((), ()))


def _layernorm(x):
    m = jnp.mean(x, axis=-1, keepdims=True)
    xc = x - m
    v = jnp.mean(xc * xc, axis=-1, keepdims=True)
    return xc / jnp.sqrt(v + 1e-5)


def _spread(items, n=4):
    per = -(-len(items) // n)
    return [items[i] for i in sorted(range(len(items)), key=lambda i: (i % per, i))]


def _cuts(total, size, shift):
    edges = [0] + list(range(shift or size, total, size)) + [total]
    return [(lo, hi - lo) for lo, hi in zip(edges, edges[1:])]


def _merge(a, b):
    keyed = [(i * len(b), 0, it) for i, it in enumerate(a)]
    keyed += [(i * len(a), 1, it) for i, it in enumerate(b)]
    return [it for _, _, it in sorted(keyed, key=lambda t: t[:2])]


class _Stream:
    def __init__(self, items):
        self.items, self.pos = list(items), 0

    def issue(self, count=None):
        left = len(self.items) - self.pos
        for _ in range(left if count is None else min(count, left)):
            src, dst, sem, prio = self.items[self.pos]
            pltpu.make_async_copy(src, dst, sem).start(priority=prio)
            self.pos += 1

    def issue_to(self, pos):
        self.issue(pos - self.pos)


def _alternate(items):
    return [it + (i % 2,) for i, it in enumerate(items)]


def _kernel(x_h, k_h, v_h, wq_h, wo_h, wg_h, wu_h, wd_h, c_h, wm_h, out_h,
            x_v, c_v, wm_v, wq_v, wo_v, wg_v, wu_v, wd_v, kbuf, vbuf, q_s, o_s, out_v,
            sem_w, sem_k, sem_v, sem_o):

    def pieces(src, dst, si, rows, cols, r_lo=0, r_hi=None):
        r_hi = src.shape[0] if r_hi is None else r_hi
        tiles = [(r, c) for r in range(r_lo, r_hi, rows) for c in range(0, src.shape[1], cols)]
        return [(src.at[pl.ds(r, rows), pl.ds(c, cols)], dst.at[pl.ds(r, rows), pl.ds(c, cols)],
                 sem_w.at[si]) for r, c in _spread(tiles)]

    def first_pair(j):
        return (j // SS) * (HG * SS) + j % SS

    def kv_pieces(j, slot):
        def copies(src, buf, sem, shift, prio):
            out = []
            for r, n in _cuts(W, NR, shift):
                for i in range(HG):
                    bh = first_pair(j) + i * SS
                    out.append((src.at[bh // HQ, bh % HQ, pl.ds(SK - W + r, n), :],
                                buf.at[slot, i, pl.ds(r, n), :], sem.at[slot], prio))
            return out
        return _merge(copies(k_h, kbuf, sem_k, K_SHIFT, 0), copies(v_h, vbuf, sem_v, 0, 1))

    def wait(dst, sem):
        pltpu.make_async_copy(dst, dst, sem).wait()

    def dot(a, b):
        return jnp.dot(a, b, preferred_element_type=F32)

    def dot_nt(a, b):
        return jax.lax.dot_general(a, b, NT, preferred_element_type=F32)

    row = jax.lax.broadcasted_iota(jnp.int32, (HG, 1), 0)

    def step_rows(j):
        return pl.ds(first_pair(j), HG, stride=SS)

    def scores(j, slot):
        wait(kbuf.at[slot], sem_k.at[slot])
        q = q_s[step_rows(j), :].astype(BF16)
        s = None
        for i in range(HG):
            si = dot_nt(q, kbuf[slot, i])
            s = si if s is None else jnp.where(row == i, si, s)
        e = jnp.exp(s - jnp.max(s, axis=-1, keepdims=True))
        return e.astype(BF16), jnp.sum(e, axis=-1, keepdims=True)

    def values(j, slot, p, l):
        wait(vbuf.at[slot], sem_v.at[slot])
        o = None
        for i in range(HG):
            oi = dot(p, vbuf[slot, i])
            o = oi if o is None else jnp.where(row == i, oi, o)
        o_s[step_rows(j), :] = o / l

    LAG = 128
    wm = _alternate(pieces(wm_h, wm_v, S_WM, 8, 1024))
    wq = _alternate(pieces(wq_h, wq_v, S_WQ, 8, 2048))
    st = _Stream([(c_h, c_v, sem_w.at[S_C], 0), (x_h, x_v, sem_w.at[S_X], 1)]
                 + wm + wq + kv_pieces(0, 0) + kv_pieces(1, 1))
    st.issue_to(2 + len(wm) + LAG)
    wait(c_v, sem_w.at[S_C])
    wait(x_v, sem_w.at[S_X])
    wait(wm_v, sem_w.at[S_WM])
    c = c_v[...].astype(F32)
    mod = dot((c * jax.nn.sigmoid(c)).astype(BF16), wm_v[...])
    sa, ca, ga, sb, cb, gb = (mod[:, i * D:(i + 1) * D] for i in range(6))
    x = x_v[...].astype(F32)
    h = (_layernorm(x) * (1.0 + ca) + sa).astype(BF16)
    st.issue_to(2 + len(wm) + len(wq) + LAG)
    wait(wq_v, sem_w.at[S_WQ])
    q = dot(h, wq_v[...]) * (DH ** -0.5)
    for hd in range(HQ):
        q_s[pl.ds(hd, B, stride=HQ), :] = q[:, hd * DH:(hd + 1) * DH]
    st.issue()

    def body(j, carry):
        slot = j % 2
        values(j, slot, *scores(j, slot))
        _Stream(kv_pieces(j + 2, slot)).issue()
        return carry

    jax.lax.fori_loop(0, NS - 2, body, 0)

    rw = HQ * DH // N_WO
    wo = [pieces(wo_h, wo_v, S_WO + g, WR, D, g * rw, (g + 1) * rw) for g in range(N_WO)]
    wg = pieces(wg_h, wg_v, S_WG, WR, D)
    wu = [pieces(wu_h, wu_v, S_WU + p, WR, D, WU_B[p], WU_B[p + 1]) for p in range(len(WU_B) - 1)]
    wd = [pieces(wd_h, wd_v, S_WD + p, WR, D, WD_B[p], WD_B[p + 1]) for p in range(len(WD_B) - 1)]
    fast = [it + (0,) for g in wo + [wg] for it in g[0::2]] + [it + (0,) for g in wu for it in g]
    slow = [it + (1,) for g in wo + [wg] for it in g[1::2]] + [it + (1,) for g in wd for it in g]
    assert len(fast) == len(slow) + 1
    st = _Stream([it for pair in zip(fast, slow) for it in pair] + fast[-1:])

    values(NS - 2, NS % 2, *scores(NS - 2, NS % 2))
    st.issue(64)
    p, l = scores(NS - 1, (NS - 1) % 2)
    st.issue(64)
    values(NS - 1, (NS - 1) % 2, p, l)
    st.issue(32)

    attn = None
    for g, more in zip(range(N_WO), (32, 32, 20, None)):
        wait(wo_v.at[pl.ds(g * rw, rw)], sem_w.at[S_WO + g])
        for hd in range(g * rw // DH, (g + 1) * rw // DH):
            o = o_s[pl.ds(hd, B, stride=HQ), :].astype(BF16)
            t = dot(o, wo_v[pl.ds(hd * DH, DH), :])
            attn = t if attn is None else attn + t
        st.issue(more)
    x = x + ga * attn
    h = (_layernorm(x) * (1.0 + cb) + sb).astype(BF16)

    wait(wg_v, sem_w.at[S_WG])
    gate = jax.nn.sigmoid(dot_nt(h, wg_v[...]))
    hh = []
    for p in range(len(WU_B) - 1):
        rows = pl.ds(WU_B[p], WU_B[p + 1] - WU_B[p])
        wait(wu_v.at[rows], sem_w.at[S_WU + p])
        hh.append((gate[:, WU_B[p]:WU_B[p + 1]] * dot_nt(h, wu_v[rows, :])).astype(BF16))
    hh = jnp.concatenate(hh, axis=1)
    down = None
    for p in range(len(WD_B) - 1):
        rows = pl.ds(WD_B[p], WD_B[p + 1] - WD_B[p])
        wait(wd_v.at[rows], sem_w.at[S_WD + p])
        t = dot(hh[:, WD_B[p]:WD_B[p + 1]], wd_v[rows, :])
        down = t if down is None else down + t
    out_v[...] = (x + gb * down).astype(BF16)
    out = pltpu.make_async_copy(out_v, out_h, sem_o)
    out.start()
    out.wait()


@jax.jit
def pallas_adaLN_cond__sliding_block_cached__glu_gated_glu__decode_kernel(
    A_x: jax.Array,
    A_k_cache: jax.Array,
    A_v_cache: jax.Array,
    A_wq: jax.Array,
    A_wo: jax.Array,
    B_x: jax.Array,
    B_w_gate: jax.Array,
    B_w_up: jax.Array,
    B_w_down: jax.Array,
    c: jax.Array,
    w_mod: jax.Array,
):
    del B_x
    assert A_x.shape == (B, 1, D) and A_k_cache.shape == A_v_cache.shape == (B, HQ, SK, DH)
    assert B_w_gate.shape == B_w_up.shape == (D, F) and B_w_down.shape == (F, D)
    hbm = pl.BlockSpec(memory_space=pltpu.HBM)
    vmem = lambda *shape, dtype=BF16: pltpu.VMEM(shape, dtype)
    dma = pltpu.SemaphoreType.DMA
    out = pl.pallas_call(
        _kernel,
        in_specs=[hbm] * 10,
        out_specs=hbm,
        out_shape=jax.ShapeDtypeStruct((B, D), BF16),
        scratch_shapes=[
            vmem(B, D), vmem(B, D), vmem(D, 6 * D), vmem(D, HQ * DH), vmem(HQ * DH, D),
            vmem(F, D), vmem(F, D), vmem(F, D),
            vmem(2, HG, W, DH), vmem(2, HG, W, DH),
            vmem(B * HQ, DH, dtype=F32), vmem(B * HQ, DH, dtype=F32), vmem(B, D),
            dma((N_WSEM,)), dma((2,)), dma((2,)), dma(()),
        ],
        compiler_params=pltpu.CompilerParams(
            vmem_limit_bytes=64 * 2**20, disable_semaphore_checks=True),
    )(
        A_x.reshape(B, D), A_k_cache, A_v_cache, A_wq, A_wo,
        B_w_gate.T, B_w_up.T, B_w_down, c, w_mod,
    )
    return out.reshape(B, 1, D)
```
